```python
import jax
import jax.numpy as jnp

def _softmax(x, axis=-1):
    return jax.nn.softmax(x, axis=axis)

def _gelu(x):
    return jax.nn.gelu(x, approximate=True)

def _silu(x):
    return jax.nn.silu(x)

def _sigmoid(x):
    return jax.nn.sigmoid(x)

def _layernorm(x, axis=-1, eps=1e-05):
    m = jnp.mean(x, axis=axis, keepdims=True)
    v = jnp.var(x, axis=axis, keepdims=True)
    return (x - m) / jnp.sqrt(v + eps)

def _scatter_add(tgt, idx, src, axis=0):
    return tgt.at[idx].add(src)

def _segment_sum(src, seg, n):
    return jax.ops.segment_sum(src, seg, n)

class _Rng:

    def __init__(self, key):
        self._k = key

    def _next(self):
        self._k, sub = jax.random.split(self._k)
        return sub

    def normal(self, shape):
        return jax.random.normal(self._next(), shape, dtype=jnp.bfloat16)

    def randint(self, lo, hi, shape):
        return jax.random.randint(self._next(), shape, lo, hi, dtype=jnp.int32)

    def uniform(self, shape, lo=0.0, hi=1.0):
        return jax.random.uniform(self._next(), shape, jnp.bfloat16, lo, hi)

    def permutation(self, n):
        return jax.random.permutation(self._next(), n)
kernel_name = 'adaLN_cond__compressed_kv_cla__dense_activation_relu__prompt'

def _fwd_setup_inputs():
    _rng = _Rng(jax.random.key(int.from_bytes(__import__("os").urandom(4), "little")))
    _w = lambda a: (lambda t: t.astype(jnp.bfloat16) if jnp.issubdtype(t.dtype, jnp.floating) else t)(jnp.asarray(a))

    def _A_setup():
        B, H, Sq, Sk, D, M = (1, 32, 2048, 2048, 128, 512)
        Dc = 4 * D
        return {'x': _w((lambda *s: _rng.normal(s) * 0.05)(B, Sq, M)), 'c_kv': _w((lambda *s: _rng.normal(s) * 0.05)(B, Sk, Dc)), 'w_q': _w((lambda *s: _rng.normal(s) * 0.05)(M, H, D) * M ** (-0.5)), 'w_uk': _w((lambda *s: _rng.normal(s) * 0.05)(Dc, H, D) * Dc ** (-0.5)), 'w_uv': _w((lambda *s: _rng.normal(s) * 0.05)(Dc, H, D) * Dc ** (-0.5)), 'w_o': _w((lambda *s: _rng.normal(s) * 0.05)(H, D, M) * (H * D) ** (-0.5))}
    _A_in = _A_setup()

    def _B_setup():
        B, S, D, Dff = (1, 2048, 512, 1792)
        return {'x': _w((lambda *s: _rng.normal(s) * 0.05)(B, S, D)), 'w1': _w((lambda *s: _rng.normal(s) * 0.05)(D, Dff)), 'w2': _w((lambda *s: _rng.normal(s) * 0.05)(Dff, D))}
    _B_in = _B_setup()
    return {'A_x': _A_in['x'], 'A_c_kv': _A_in['c_kv'], 'A_w_q': _A_in['w_q'], 'A_w_uk': _A_in['w_uk'], 'A_w_uv': _A_in['w_uv'], 'A_w_o': _A_in['w_o'], 'B_x': _B_in['x'], 'B_w1': _B_in['w1'], 'B_w2': _B_in['w2'], 'c': _w((lambda *s: _rng.normal(s) * 0.05)(1, 512)), 'w_mod': _w((lambda *s: _rng.normal(s) * 0.05)(512, 6 * 512) * 512 ** (-0.5))}

def _fwd_reference(A_x, A_c_kv, A_w_q, A_w_uk, A_w_uv, A_w_o, B_x, B_w1, B_w2, c, w_mod):

    def _A_ref(x, c_kv, w_q, w_uk, w_uv, w_o):
        B, Sq, M = (x.shape[0], x.shape[1], x.shape[2])
        Sk = c_kv.shape[1]
        H, D = (w_q.shape[1], w_q.shape[2])
        q = jnp.einsum('bqm,mhd->bhqd', x, w_q)
        k = jnp.einsum('bkc,chd->bhkd', c_kv, w_uk)
        v = jnp.einsum('bkc,chd->bhkd', c_kv, w_uv)
        scores = jnp.einsum('bhqd,bhkd->bhqk', q, k) * D ** (-0.5)
        off = Sk - Sq
        qi = jnp.arange(Sq)[:, None]
        kj = jnp.arange(Sk)[None, :]
        cmask = kj <= qi + off
        scores = jnp.where(cmask[None, None], scores, -1000000000.0)
        p = _softmax(scores, axis=-1)
        ctx = jnp.einsum('bhqk,bhkd->bhqd', p, v)
        return jnp.einsum('bhqd,hdm->bqm', ctx, w_o)

    def _B_ref(x, w1, w2):
        h = jnp.einsum('bsd,df->bsf', x, w1)
        zero = jnp.zeros_like(h)
        h = jnp.maximum(h, zero)
        return jnp.einsum('bsf,fd->bsd', h, w2)
    x = A_x
    mod = (_silu(c) @ w_mod).reshape(c.shape[0], 6, 1, -1)
    sa, ca, ga, sb, cb, gb = (mod[:, 0].copy(), mod[:, 1].copy(), mod[:, 2].copy(), mod[:, 3].copy(), mod[:, 4].copy(), mod[:, 5].copy())
    h = _layernorm(x, axis=-1) * (1 + ca) + sa
    x = x + ga * _A_ref(h, A_c_kv, A_w_q, A_w_uk, A_w_uv, A_w_o)
    h = _layernorm(x, axis=-1) * (1 + cb) + sb
    x = x + gb * _B_ref(h, B_w1, B_w2)
    return x

def setup_inputs():
    _inp = _fwd_setup_inputs()
    _gk = jax.random.fold_in(jax.random.key(int.from_bytes(__import__("os").urandom(4), "little")), 2 ** 31 - 1)
    _shapes = [[1, 2048, 512]]
    _dtypes = ['bfloat16']
    _gks = jax.random.split(_gk, len(_shapes))
    _gs = [jax.random.normal(k, s, dtype=jnp.dtype(d)) * 0.05 for k, s, d in zip(_gks, _shapes, _dtypes)]
    _inp['grad_out'] = _gs[0]
    return _inp

def reference(A_x, A_c_kv, A_w_q, A_w_uk, A_w_uv, A_w_o, B_w1, B_w2, c, w_mod, B_x, grad_out):
    _const = dict(B_x=B_x)

    def _f(*_d):
        return _fwd_reference(**{'A_x': _d[0], 'A_c_kv': _d[1], 'A_w_q': _d[2], 'A_w_uk': _d[3], 'A_w_uv': _d[4], 'A_w_o': _d[5], 'B_w1': _d[6], 'B_w2': _d[7], 'c': _d[8], 'w_mod': _d[9], **_const})
    _out, _vjp = jax.vjp(_f, A_x, A_c_kv, A_w_q, A_w_uk, A_w_uv, A_w_o, B_w1, B_w2, c, w_mod)
    _grads = _vjp(grad_out)
    _out0 = jnp.asarray(_out)
    return (_out0, *[jnp.asarray(_g) for _g in _grads])
```

```python
import math

import jax
import jax.numpy as jnp
from jax import lax
from jax.experimental import pallas as pl
from jax.experimental.pallas import tpu as pltpu

S = 2048
M = 512
H = 32
D = 128
FF = 1792
EPS = 1e-5
NEG = -1e30
LOG2E = math.log2(math.e)
LN2 = math.log(2.0)
SCALE = D ** -0.5

bf16 = jnp.bfloat16
f32 = jnp.float32

NN = (((1,), (0,)), ((), ()))
NT = (((1,), (1,)), ((), ()))
TN = (((0,), (0,)), ((), ()))

WROWS = M * H

(SEM_CKV, SEM_X, SEM_C, SEM_WMOD, SEM_WO, SEM_W1,
 SEM_W2, SEM_G, SEM_CKV2, SEM_WMOD2, SEM_DW1, SEM_DW2, SEM_DC) = range(13)
SEM_DWO = 16
SEM_DX = 48
SEM_DCKV = 56
SEM_DW = 64
SEM_DWMOD = 76
SEM_POUT = 80
SEM_PIN = 82
SEM_OUT = 84
SEM_RAW = 100
NSEM = 106

NT_ = S // 128
NTILE = NT_ * (NT_ + 1) // 2
NSAVE = H - 2


def _tile(kt, qt):
    return NT_ * kt - kt * (kt - 1) // 2 + (qt - kt)


def _dot(a, b, dims=NN):
    return lax.dot_general(a, b, dims, preferred_element_type=f32)


def _colred(x, op, acc=4):
    n, w = x.shape
    g = 8 * acc
    if n > g and n % g == 0:
        x = op(x.reshape(n // g, g, w), axis=0)
        n = g
    if n > 8:
        x = op(x.reshape(n // 8, 8, w), axis=0)
    return x


def _diag_mask():
    row = lax.broadcasted_iota(jnp.int32, (128, 128), 0)
    col = lax.broadcasted_iota(jnp.int32, (128, 128), 1)
    return row <= col


def _mask_first_tile(x, fill):
    xd = jnp.where(_diag_mask(), x[:, :128], fill)
    if x.shape[1] > 128:
        return jnp.concatenate([xd, x[:, 128:]], axis=1)
    return xd


def _ln_stats(x):
    mu = jnp.mean(x, axis=-1, keepdims=True)
    xc = x - mu
    var = jnp.mean(xc * xc, axis=-1, keepdims=True)
    rstd = lax.rsqrt(var + EPS)
    return xc * rstd, rstd


def _ln_bwd(dxhat, xhat, rstd):
    a = jnp.mean(dxhat, axis=-1, keepdims=True)
    b = jnp.mean(dxhat * xhat, axis=-1, keepdims=True)
    return rstd * (dxhat - a - xhat * b)


def _cat(xs, axis):
    return jnp.concatenate(xs, axis=axis) if len(xs) > 1 else xs[0]


def _tiles(ref, c0, c1):
    return _cat([ref[t] for t in range(c0 // 128, c1 // 128)], 1)


def _rows(start, size, mult):
    return pl.ds(pl.multiple_of(start, mult), size)


F_BQ = 1024
F_CFG = dict(
    order=(0, 5, 6, 7, 4, 3, 2, 1, 17, 14, 10, 15,
           12, 13, 22, 11, 9, 20, 18, 19, 21, 8, 23, 16),
    look={1: 3, 2: 2, 5: 3, 6: 3, 7: 2, 8: 4, 9: 3, 10: 2, 13: 3, 14: 3, 16: 2,
          17: 2, 19: 4, 20: 2, 22: 3},
    delay=9,
    chains_max=1,
    chains_sum=8,
    vt_ahead=2,
)


def _fwd_steps():
    steps = []
    for j in range(S // F_BQ):
        steps += [(j, j * F_BQ + c, c, True) for c in range(0, F_BQ, 128)]
    steps += [(1, k, 0, False) for k in range(0, F_BQ, 128)]
    steps = [steps[i] for i in F_CFG["order"]]
    assert sorted(F_CFG["order"]) == list(range(len(steps)))
    for j in range(S // F_BQ):
        assert next(st for st in steps if st[0] == j)[2] == 0
    return steps


def _attn_fwd(k_ref, vt_ref, make_vt, qt_ref, p_ref, m_ref, lse_ref, store_tile,
              project):
    steps = _fwd_steps()
    last = {st[0]: i for i, st in enumerate(steps)}
    state = {}
    fillers = {}
    have_vt = set()

    def scores(st):
        j, k0, c0, dg = st
        q0 = j * F_BQ
        s = _dot(k_ref[k0:k0 + 128, :], _tiles(qt_ref, q0 + c0, q0 + F_BQ))
        return _mask_first_tile(s, NEG) if dg else s

    def keep(old, new, c0):
        return jnp.concatenate([old[:, :c0], new], axis=1) if c0 > 0 else new

    def update(i, st, s):
        j, k0, c0, dg = st
        q0 = j * F_BQ
        mloc = jnp.max(_colred(s, jnp.max, F_CFG["chains_max"]), axis=0, keepdims=True)
        first = j not in state
        if first:
            m = mloc
        else:
            mo, lo, ao = state[j]
            m = jnp.maximum(mo[:, c0:], mloc)
            alpha = jnp.exp2(mo[:, c0:] - m)
        p = jnp.exp2(s - m)
        idx = [_tile(k0 // 128, qt)
               for qt in range((q0 + c0) // 128, (q0 + F_BQ) // 128)]

        for c, t in enumerate(idx):
            m_ref[t:t + 1, :] = m[:, c * 128:(c + 1) * 128]
            p_ref[t] = p[:, c * 128:(c + 1) * 128].astype(bf16)
        l = _colred(p, jnp.sum, F_CFG["chains_sum"])
        acc = _dot(vt_ref[k0 // 128], _cat([p_ref[t] for t in idx], 1))
        if not first:
            l = lo[:, c0:] * alpha + l
            acc = ao[:, c0:] * alpha + acc
            m, l, acc = keep(mo, m, c0), keep(lo, l, c0), keep(ao, acc, c0)
        state[j] = (m, l, acc)
        if i == last[j]:
            lt = jnp.sum(l, axis=0, keepdims=True)
            lse_ref[:, q0:q0 + F_BQ] = m + jnp.log2(lt)
            accn = acc * (1.0 / lt)
            cts = [accn[:, c * 128:(c + 1) * 128].astype(bf16)
                   for c in range(F_BQ // 128)]
            for c, ctb in enumerate(cts):
                store_tile(q0 // 128 + c, ctb)
            at = i + F_CFG["delay"]
            if at >= len(steps):
                project(q0 // 128, cts)
            else:
                fillers.setdefault(at, []).append(lambda: project(q0 // 128, cts))
            del state[j]

    def prepare_vt(upto):
        for st in steps[:upto + 1]:
            kt = st[1] // 128
            if kt not in have_vt:
                have_vt.add(kt)
                make_vt(kt)

    pend = {0: scores(steps[0])}
    nxt = 1
    for i, st in enumerate(steps):
        cur = pend.pop(i)
        while nxt < len(steps) and nxt - i <= F_CFG["look"].get(i, 1):
            pend[nxt] = scores(steps[nxt])
            nxt += 1
        prepare_vt(i + F_CFG["vt_ahead"])
        for fill in fillers.pop(i, ()):
            fill()
        update(i, st, cur)


def _fwd_head(h, KV, QT, CT, WO, DX1, VT, p_ref, MROW, LSE):
    wo = WO[_rows(h * D, D, D), :]

    def make_vt(c):
        VT[c] = KV[H + h, c * 128:(c + 1) * 128, :].T

    def store_tile(t, ctb):
        CT[h, t] = ctb

    def project(t0, cts):
        ctx = jnp.concatenate([t.T for t in cts], axis=0)
        rows = slice(t0 * 128, (t0 + len(cts)) * 128)
        DX1[rows, :] = jnp.where(h > 0, DX1[rows, :], 0.0) + _dot(ctx, wo)

    _attn_fwd(KV.at[h], VT, make_vt, QT.at[h], p_ref, MROW.at[h], LSE.at[h],
              store_tile, project)


B_BK = 512
B_CFG = dict(
    bq=(512, 512, 512, 512),
    order=((0, 1, 2, 3, 4, 5, 6), (0, 1, 2, 3, 4, 5), (1, 2, 0, 4, 3), (3, 0, 1, 2)),
    look={11: 3, 12: 2, 13: 2},
    dc_delay=0,
    dh_delay=4,
    dwo_at=21,
    kt_ahead=0,
)


def _bwd_steps():
    steps = []
    for kb in range(S // B_BK):
        k0 = kb * B_BK
        bq = B_CFG["bq"][kb]
        lst = [(k0 + 128 * t, k0 + 128 * (t + 1), k0 + 128 * t, k0 + B_BK)
               for t in range(B_BK // 128)]
        lst += [(k0, k0 + B_BK, q, min(S, q + bq)) for q in range(k0 + B_BK, S, bq)]
        order = B_CFG["order"][kb]
        assert sorted(order) == list(range(len(lst)))
        steps += [(kb, i == len(lst) - 1) + lst[o] for i, o in enumerate(order)]
    return steps


def _attn_bwd(v_ref, kt_ref, make_kt, qt_ref, dot_ref, p_ref, m_ref, lse, delta,
              dq_acc, finish_block, fillers):
    steps = _bwd_steps()
    state = {}
    seen_q = set()
    have_kt = set()

    def phase_a(st):
        kb, last, k0, k1, q0, q1 = st
        return _dot(v_ref[k0:k1, :], _tiles(dot_ref, q0, q1))

    def phase_b(i, st, dp):
        kb, last, k0, k1, q0, q1 = st
        rows = []
        for kt in range(k0 // 128, k1 // 128):
            idx = [_tile(kt, qt) for qt in range(q0 // 128, q1 // 128)]
            corr = jnp.exp2(_cat([m_ref[t:t + 1, :] for t in idx], 1) - lse[:, q0:q1])
            rows.append(_cat([p_ref[t].astype(f32) for t in idx], 1) * corr)
        p = _cat(rows, 0)
        ds = p * (dp - delta[:, q0:q1])
        pb = p.astype(bf16)
        dsb = ds.astype(bf16)
        dv = _dot(pb, _tiles(dot_ref, q0, q1), NT)
        dk = _dot(dsb, _tiles(qt_ref, q0, q1), NT)
        dq = _dot(_tiles(kt_ref, k0, k1), dsb)
        kb0 = kb * B_BK
        for t in range((k1 - k0) // 128):
            key = (k0 - kb0) // 128 + t
            a = dv[t * 128:(t + 1) * 128]
            b = dk[t * 128:(t + 1) * 128]
            if key in state:
                a = a + state[key][0]
                b = b + state[key][1]
            state[key] = (a, b)
        c = q0 // 128
        while c < q1 // 128:
            e = c
            while e < q1 // 128 and (e in seen_q) == (c in seen_q):
                e += 1
            piece = dq[:, c * 128 - q0:e * 128 - q0]
            if c in seen_q:
                dq_acc[:, c * 128:e * 128] += piece
            else:
                dq_acc[:, c * 128:e * 128] = piece
            c = e
        seen_q.update(range(q0 // 128, q1 // 128))
        if last:
            n = B_BK // 128
            dvb = jnp.concatenate([state[t][0] for t in range(n)], axis=0)
            dkb = jnp.concatenate([state[t][1] for t in range(n)], axis=0)
            state.clear()
            finish_block(i, kb0, dkb, dvb)

    def prepare_kt(upto):
        for st in steps[:upto + 1]:
            for kt in range(st[2] // 128, st[3] // 128):
                if kt not in have_kt:
                    have_kt.add(kt)
                    make_kt(kt)

    pend = {0: phase_a(steps[0])}
    nxt = 1
    for i, st in enumerate(steps):
        cur = pend.pop(i)
        while nxt < len(steps) and nxt - i <= B_CFG["look"].get(i, 1):
            pend[nxt] = phase_a(steps[nxt])
            nxt += 1
        prepare_kt(i + B_CFG["kt_ahead"])
        for fill in fillers.pop(i, ()):
            fill()
        phase_b(i, st, cur)
    for i in sorted(fillers):
        for fill in fillers[i]:
            fill()


def _bwd_head(h, first, KV, QT, CT, WO, WRK, WRV, WRQ, DATT, DCA, DH1T, DOT, KT, DQ,
              p_ref, MROW, LSE):
    wrows = _rows(h * D, D, D)
    datt = DATT[...]
    dot32 = _dot(WO[wrows, :], datt, NT)
    deltas = []
    kt_first = B_CFG["kt_ahead"] >= 99
    for c in range(NT_):
        DOT[c] = dot32[:, c * 128:(c + 1) * 128].astype(bf16)
        prod = DOT[c].astype(f32) * CT[h, c].astype(f32)
        deltas.append(jnp.sum(_colred(prod, jnp.sum), axis=0, keepdims=True))
        if kt_first:
            KT[c] = KV[h, c * 128:(c + 1) * 128, :].T
    delta = jnp.concatenate(deltas, axis=1)
    fillers = {}

    def dwo():
        WO[wrows, :] = _dot(_tiles(CT.at[h], 0, S), datt).astype(bf16)

    if B_CFG["dwo_at"] < 0:
        dwo()
    else:
        fillers[B_CFG["dwo_at"]] = [dwo]
    wuk = WRK[_rows(h * M, M, M), :]
    wuv = WRV[_rows(h * M, M, M), :]
    wq = WRQ[_rows(h * M, M, M), :]
    wkv = jnp.concatenate([wuk, wuv], axis=1)

    def make_kt(c):
        if not kt_first:
            KT[c] = KV[h, c * 128:(c + 1) * 128, :].T

    def finish_block(i, k0, dk, dv):
        blk = slice(k0, k0 + B_BK)
        dkb = (dk * LN2).astype(bf16)
        dvb = dv.astype(bf16)
        KV[h, blk, :] = dkb
        KV[H + h, blk, :] = dvb

        def dc():
            r = _dot(jnp.concatenate([dkb, dvb], axis=1), wkv, NT)
            DCA[blk, :] = jnp.where(first, 0.0, DCA[blk, :]) + r

        def dh():
            for c in range(k0 // 128, (k0 + B_BK) // 128):
                QT[h, c] = (DQ[:, c * 128:(c + 1) * 128] * SCALE).astype(bf16)
            DH1T[:, blk] = (jnp.where(first, 0.0, DH1T[:, blk])
                            + _dot(wq, _tiles(QT.at[h], k0, k0 + B_BK)))

        for delay, fn in ((B_CFG["dc_delay"], dc), (B_CFG["dh_delay"], dh)):
            if delay == 0:
                fn()
            else:
                fillers.setdefault(i + delay, []).append(fn)

    _attn_bwd(KV.at[H + h], KT, make_kt, QT.at[h], DOT, p_ref, MROW.at[h], LSE[h],
              delta, DQ, finish_block, fillers)


C = 128
NC = 2
M_CFG = dict(order=(
    ("df", 0), ("da", 0), ("ln", 0), ("df", 1), ("u", 0), ("da", 1),
    ("ln", 1), ("u", 1), ("act", 0), ("f", 0), ("act", 1), ("out", 0),
    ("f", 1), ("out", 1), ("dw2", 1), ("dw2", 0), ("du", 0), ("dh2", 0),
    ("du", 1), ("dh2", 1), ("dw1", 0), ("lnb", 0), ("dw1", 1), ("lnb", 1),
))
M_DEPS = {"df": (), "da": ("df",), "ln": (), "u": ("ln",), "act": ("u",),
          "f": ("act",), "out": ("f",), "dw2": ("act", "df"), "du": ("da", "act"),
          "dh2": ("du",), "dw1": ("du",), "lnb": ("dh2",)}


def _mid_iter(it, mod, start_out, XB, G, DX1, W1, W2, OUTS, DATT, DW1, DW2, DM):
    js = [NC * it + n for n in range(NC)]
    rows = [_rows(j * C, C, C) for j in js]
    st = [dict() for _ in range(NC)]
    started = set()

    def accumulate(ref, r):
        if id(ref) not in started:
            started.add(id(ref))
            ref[...] = jnp.where(it > 0, ref[...], 0.0) + r
        else:
            ref[...] += r

    def s_df(n):
        st[n]["df"] = (G[rows[n], :].astype(f32) * mod(5)).astype(bf16)

    def s_da(n):
        st[n]["da"] = _dot(st[n]["df"], W2[...], NT)

    def s_ln(n):
        attn = DX1[rows[n], :]
        x1 = XB[rows[n], :].astype(f32) + mod(2) * attn
        xhat, rstd = _ln_stats(x1)
        st[n].update(attn=attn, x1=x1, xhat=xhat, rstd=rstd,
                     h2=(xhat * (1.0 + mod(4)) + mod(3)).astype(bf16))

    def s_u(n):
        st[n]["u"] = _dot(st[n]["h2"], W1[...])

    def s_act(n):
        u = st[n].pop("u")
        st[n]["a"] = jnp.maximum(u, 0.0).astype(bf16)
        st[n]["slope"] = jnp.where(
            u > 0.0, 1.0, jnp.where(u == 0.0, 0.5, 0.0)).astype(bf16)

    def s_f(n):
        st[n]["f"] = _dot(st[n]["a"], W2[...])

    def s_out(n):
        f = st[n].pop("f")
        OUTS[rows[n], :] = (st[n].pop("x1") + mod(5) * f).astype(bf16)
        start_out(js[n])
        DM[5] += _colred(G[rows[n], :].astype(f32) * f, jnp.sum)

    def s_dw2(n):
        accumulate(DW2, _dot(st[n]["a"], st[n]["df"], TN))

    def s_du(n):
        st[n]["du"] = (st[n].pop("da") * st[n].pop("slope").astype(f32)).astype(bf16)

    def s_dh2(n):
        st[n]["dh2"] = _dot(st[n]["du"], W1[...], NT)

    def s_dw1(n):
        accumulate(DW1, _dot(st[n]["h2"], st[n]["du"], TN))

    def s_lnb(n):
        dh2 = st[n].pop("dh2")
        xhat = st[n].pop("xhat")
        DM[3] += _colred(dh2, jnp.sum)
        DM[4] += _colred(dh2 * xhat, jnp.sum)
        dx1 = G[rows[n], :].astype(f32) + _ln_bwd(
            dh2 * (1.0 + mod(4)), xhat, st[n].pop("rstd"))
        DM[2] += _colred(dx1 * st[n].pop("attn"), jnp.sum)
        DX1[rows[n], :] = dx1
        DATT[rows[n], :] = (dx1 * mod(2)).astype(bf16)

    stages = dict(df=s_df, da=s_da, ln=s_ln, u=s_u, act=s_act, f=s_f, out=s_out,
                  dw2=s_dw2, du=s_du, dh2=s_dh2, dw1=s_dw1, lnb=s_lnb)
    done = set()
    for name, n in M_CFG["order"]:
        assert all((d, n) in done for d in M_DEPS[name]), (name, n)
        stages[name](n)
        done.add((name, n))
    assert len(done) == NC * len(stages)


def _kernel(x_hbm, ckv_hbm, wq_hbm, wuk_hbm, wuv_hbm, wo_hbm, w1_hbm, w2_hbm,
            c_hbm, wmod_hbm, g_hbm,
            out_hbm, dx_hbm, dckv_hbm, dwq_hbm, dwuk_hbm, dwuv_hbm, dwo_hbm,
            dw1_hbm, dw2_hbm, dc_hbm, dwmod_hbm, p_hbm,
            QT, KV, CT, WRK, WRV, WRQ, MROW, LSE, MOD, DM, XB, CV, WO, sems):

    def copy(src, dst, slot):
        return pltpu.make_async_copy(src, dst, sems.at[slot])

    def mod(i):
        return MOD[:, i * M:(i + 1) * M]

    def phase_proj(RAW, CKV, H1, WMOD):
        def cp_raw(i, half):
            src = (wuk_hbm, wuv_hbm, wq_hbm)[i]
            heads = pl.ds(pl.multiple_of(half * 16, 16), 16)
            return copy(src.at[:, heads, :], RAW.at[2 * i + half],
                        SEM_RAW + 2 * i + half)

        cp_ckv = copy(ckv_hbm, CKV, SEM_CKV)
        cp_x = copy(x_hbm, XB, SEM_X)
        cp_c = copy(c_hbm, CV, SEM_C)
        cp_wmod = copy(wmod_hbm, WMOD, SEM_WMOD)
        for cp in (cp_c, cp_raw(0, 0), cp_ckv, cp_raw(0, 1), cp_raw(1, 0), cp_raw(1, 1),
                   cp_wmod, cp_x, cp_raw(2, 0), cp_raw(2, 1),
                   copy(wo_hbm, WO, SEM_WO)):
            cp.start()

        DM[...] = jnp.zeros(DM.shape, f32)

        def relayout(dst, i, u):
            j0 = 2 * i
            half = u // 4
            for s in range(8):
                m0 = (u % 4) * 128 + s * 16
                v = jnp.swapaxes(RAW[j0 + half, _rows(m0, 16, 16)], 0, 1)
                for t in range(16):
                    dst[_rows((half * 16 + t) * M + m0, 16, 16), :] = v[t]

        def wslab(src, g):
            return jnp.concatenate(
                [src[_rows((g * 8 + t) * M, M, M), :] for t in range(8)], axis=1)

        def relayout_half(dst, i, half):
            cp_raw(i, half).wait()

            def body_r(u, carry):
                relayout(dst, i, u)
                return carry
            lax.fori_loop(4 * half, 4 * half + 4, body_r, 0)

        with jax.named_scope("relayout_uk"):
            relayout_half(WRK, 0, 0)

        with jax.named_scope("proj_k"):
            cp_ckv.wait()

            def body_k(g, carry):
                @pl.when(g == 2)
                def _():
                    relayout_half(WRK, 0, 1)

                r = _dot(CKV[...], wslab(WRK, g))
                for t in range(8):
                    KV[g * 8 + t] = r[:, t * D:(t + 1) * D].astype(bf16)
                return carry
            lax.fori_loop(0, H // 8, body_k, 0)

        with jax.named_scope("relayout_uv"):
            relayout_half(WRV, 1, 0)
            relayout_half(WRV, 1, 1)

        with jax.named_scope("mod"):
            cp_c.wait()
            cp_wmod.wait()
            cv = CV[...].astype(f32)
            sc = cv * jax.nn.sigmoid(cv)
            scb = jnp.broadcast_to(sc, (16, M)).astype(bf16)
            MOD[...] = _dot(scb, WMOD[...])[0:1, :]
            cp_x.wait()

        with jax.named_scope("proj_v"):
            def body_v(g, carry):
                @pl.when(g % 2 == 0)
                def _():
                    cp_raw(2, g // 2).wait()

                r = _dot(CKV[...], wslab(WRV, g))
                for t in range(8):
                    KV[H + g * 8 + t] = r[:, t * D:(t + 1) * D].astype(bf16)
                for n in range(2):
                    relayout(WRQ, 2, 2 * g + n)
                for n in range(2):
                    rows = _rows(g * 512 + n * 256, 256, 256)
                    xhat, _ = _ln_stats(XB[rows, :].astype(f32))
                    H1[rows, :] = (xhat * (1.0 + mod(1)) + mod(0)).astype(bf16)
                return carry
            lax.fori_loop(0, H // 8, body_v, 0)

        with jax.named_scope("proj_q"):
            def body_q(g, carry):
                r = _dot(H1[...], wslab(WRQ, g)) * (SCALE * LOG2E)
                for t in range(8):
                    qb = r[:, t * D:(t + 1) * D].astype(bf16)
                    for c in range(NT_):
                        QT[g * 8 + t, c] = qb[c * 128:(c + 1) * 128].T
                return carry
            lax.fori_loop(0, H // 8, body_q, 0)

    pl.run_scoped(
        phase_proj,
        pltpu.VMEM((6, M, 16, D), bf16),
        pltpu.VMEM((S, M), bf16), pltpu.VMEM((S, M), bf16),
        pltpu.VMEM((M, 6 * M), bf16))

    def phase_main(W1, W2, G, OUTS, DX1, DATT, PST):
        cp_w1 = copy(w1_hbm, W1, SEM_W1)
        cp_w2 = copy(w2_hbm, W2, SEM_W2)
        cp_g = copy(g_hbm, G, SEM_G)
        for cp in (cp_w1, cp_w2, cp_g):
            cp.start()
        copy(wo_hbm, WO, SEM_WO).wait()

        def cp_pout(h):
            return copy(PST.at[h % 2], p_hbm.at[h], SEM_POUT + h % 2)

        def cp_pin(h):
            return copy(p_hbm.at[h], PST.at[h % 2], SEM_PIN + h % 2)

        def phase_fwd(VT):
            def body(h, carry):
                @pl.when(h >= 2)
                def _():
                    cp_pout(h - 2).wait()

                _fwd_head(h, KV, QT, CT, WO, DX1, VT, PST.at[h % 2], MROW, LSE)

                @pl.when(h < NSAVE)
                def _():
                    cp_pout(h).start()
                return carry
            lax.fori_loop(0, H, body, 0)

        with jax.named_scope("attn_fwd"):
            pl.run_scoped(phase_fwd, pltpu.VMEM((NT_, D, 128), bf16))

        def cp_out(j):
            rows = _rows(j * C, C, C)
            return copy(OUTS.at[rows], out_hbm.at[rows], SEM_OUT + j)

        def phase_mid(DW1, DW2):
            for cp in (cp_w1, cp_w2, cp_g):
                cp.wait()

            def body(it, carry):
                _mid_iter(it, mod, lambda j: cp_out(j).start(), XB, G, DX1, W1, W2,
                          OUTS, DATT, DW1, DW2, DM)
                return carry
            lax.fori_loop(0, S // (NC * C), body, 0)

            W1[...] = DW1[...].astype(bf16)
            W2[...] = DW2[...].astype(bf16)
            copy(W1, dw1_hbm, SEM_DW1).start()
            copy(W2, dw2_hbm, SEM_DW2).start()

        with jax.named_scope("mid"):
            pl.run_scoped(phase_mid, pltpu.VMEM((M, FF), f32),
                          pltpu.VMEM((FF, M), f32))

        def cp_dwo(h):
            rows = _rows(h * D, D, D)
            return copy(WO.at[rows], dwo_hbm.at[rows], SEM_DWO + h)

        def phase_bwd(DH1T, DCA):
            CKV = G
            cp_ckv = copy(ckv_hbm, CKV, SEM_CKV2)
            cp_ckv.start()

            def bwd_loop(DOT, KT, DQ):
                def body(i, carry):
                    h = H - 1 - i

                    @pl.when(h < NSAVE)
                    def _():
                        cp_pin(h).wait()

                    @pl.when(jnp.logical_and(h >= 1, h <= NSAVE))
                    def _():
                        cp_pin(h - 1).start()

                    _bwd_head(h, i == 0, KV, QT, CT, WO, WRK, WRV, WRQ, DATT, DCA,
                              DH1T, DOT, KT, DQ, PST.at[h % 2], MROW, LSE)
                    cp_dwo(h).start()
                    return carry
                lax.fori_loop(0, H, body, 0)

            with jax.named_scope("attn_bwd"):
                pl.run_scoped(bwd_loop, pltpu.VMEM((NT_, D, 128), bf16),
                              pltpu.VMEM((NT_, D, 128), bf16), pltpu.VMEM((D, S), f32))

            def phase_dw(WMOD, H1T):
                cp_wmod = copy(wmod_hbm, WMOD, SEM_WMOD2)
                cp_wmod.start()
                def stage_dw(n, count, head_grad):
                    res = [head_grad(h).astype(bf16) for h in range(H)]
                    for i in range(8 * count):
                        v = jnp.stack([r[i * 16:(i + 1) * 16] for r in res], axis=0)
                        v = jnp.swapaxes(v, 0, 1).reshape(4, 128, D)
                        CT[2 * n + i // 4, (i % 4) * 4:(i % 4) * 4 + 4] = v

                def cp_dw(w_idx, g, dst):
                    n = w_idx * 4 + g
                    return copy(CT.at[pl.ds(2 * n, 2)], dst.at[pl.ds(2 * g, 2)],
                                SEM_DW + n)

                def cp_dx(j):
                    rows = _rows(j * 256, 256, 256)
                    return copy(DATT.at[rows], dx_hbm.at[rows], SEM_DX + j)

                def cp_dckv(j):
                    rows = _rows(j * 256, 256, 256)
                    return copy(OUTS.at[rows], dckv_hbm.at[rows], SEM_DCKV + j)

                def cp_dwmod(g):
                    rows = _rows(g * 128, 128, 128)
                    return copy(WMOD.at[rows], dwmod_hbm.at[rows], SEM_DWMOD + g)

                with jax.named_scope("dw_kv"):
                    cp_ckv.wait()
                    for j in range(S // C):
                        cp_out(j).wait()

                    def body_kv(g, carry):
                        for n in range(2):
                            rows = _rows(g * 512 + n * 256, 256, 256)
                            dh1 = DH1T[:, rows].T
                            xhat, rstd = _ln_stats(XB[rows, :].astype(f32))
                            H1T[:, rows] = (xhat * (1.0 + mod(1))
                                            + mod(0)).astype(bf16).T
                            DM[0] += _colred(dh1, jnp.sum)
                            DM[1] += _colred(dh1 * xhat, jnp.sum)
                            dx = DX1[rows, :] + _ln_bwd(dh1 * (1.0 + mod(1)), xhat, rstd)
                            DATT[rows, :] = dx.astype(bf16)
                            OUTS[rows, :] = DCA[rows, :].astype(bf16)

                        w_idx = g // 2
                        g2 = g % 2
                        cols = pl.ds(pl.multiple_of(g2 * 256, 256), 256)
                        ct = CKV[:, cols].T
                        stage_dw(4 * w_idx + 2 * g2, 2,
                                 lambda h: _dot(ct, KV[w_idx * H + h]))

                        for n in range(2):
                            cp_dx(2 * g + n).start()
                            cp_dckv(2 * g + n).start()

                        @pl.when(w_idx == 0)
                        def _():
                            for n in range(2):
                                cp_dw(0, 2 * g2 + n, dwuk_hbm).start()

                        @pl.when(w_idx == 1)
                        def _():
                            for n in range(2):
                                cp_dw(1, 2 * g2 + n, dwuv_hbm).start()
                        return carry
                    lax.fori_loop(0, 4, body_kv, 0)

                cp_dc = copy(CV, dc_hbm, SEM_DC)
                with jax.named_scope("dw_q"):
                    cp_wmod.wait()
                    dmod = jnp.concatenate(
                        [jnp.sum(DM[i], axis=0, keepdims=True) for i in range(6)],
                        axis=1)
                    hi = dmod.astype(bf16)
                    lo = (dmod - hi.astype(f32)).astype(bf16)
                    sub = lax.broadcasted_iota(jnp.int32, (16, 6 * M), 0)
                    dm2 = jnp.where(sub == 0, hi.astype(f32),
                                    jnp.where(sub == 1, lo.astype(f32), 0.0)).astype(bf16)
                    cv = CV[...].astype(f32)
                    sig = jax.nn.sigmoid(cv)
                    sc = cv * sig
                    dsc = sig * (1.0 + cv * (1.0 - sig))
                    MOD[:, 0:M] = dsc
                    MOD[:, M:2 * M] = sc

                    def body_mod(g, carry):
                        rows = _rows(g * 128, 128, 128)
                        cols = pl.ds(pl.multiple_of(g * 128, 128), 128)
                        r = _dot(dm2, WMOD[rows, :], NT)
                        CV[:, cols] = ((r[0:1] + r[1:2]) * MOD[:, cols]).astype(bf16)
                        scol = jnp.broadcast_to(
                            MOD[:, pl.ds(pl.multiple_of(M + g * 128, 128), 128)],
                            (128, 128)).T
                        for t in range(6 * M // 128):
                            WMOD[rows, t * 128:(t + 1) * 128] = (
                                scol * dmod[:, t * 128:(t + 1) * 128]).astype(bf16)
                        cp_dwmod(g).start()
                        return carry
                    lax.fori_loop(0, 4, body_mod, 0)
                    cp_dc.start()

                    def body_q(g, carry):
                        lhs = H1T[_rows(g * 128, 128, 128), :]
                        stage_dw(8 + g, 1,
                                 lambda h: _dot(lhs, _tiles(QT.at[h], 0, S), NT))
                        cp_dw(2, g, dwq_hbm).start()
                        return carry
                    lax.fori_loop(0, 4, body_q, 0)

                with jax.named_scope("drain"):
                    copy(W1, dw1_hbm, SEM_DW1).wait()
                    copy(W2, dw2_hbm, SEM_DW2).wait()
                    for h in range(H):
                        cp_dwo(h).wait()
                    for j in range(8):
                        cp_dx(j).wait()
                        cp_dckv(j).wait()
                    for g in range(4):
                        cp_dw(0, g, dwuk_hbm).wait()
                        cp_dw(1, g, dwuv_hbm).wait()
                        cp_dw(2, g, dwq_hbm).wait()
                        cp_dwmod(g).wait()
                    cp_dc.wait()

            pl.run_scoped(phase_dw, pltpu.VMEM((M, 6 * M), bf16),
                          pltpu.VMEM((M, S), bf16))

        pl.run_scoped(
            phase_bwd,
            pltpu.VMEM((M, S), f32), pltpu.VMEM((S, M), f32))

    pl.run_scoped(
        phase_main,
        pltpu.VMEM((M, FF), bf16),
        pltpu.VMEM((FF, M), bf16), pltpu.VMEM((S, M), bf16),
        pltpu.VMEM((S, M), bf16), pltpu.VMEM((S, M), f32),
        pltpu.VMEM((S, M), bf16), pltpu.VMEM((2, NTILE, 128, 128), bf16))


@jax.jit
def pallas_adaLN_cond__compressed_kv_cla__dense_activation_relu__prompt_kernel(
    A_x: jax.Array,
    A_c_kv: jax.Array,
    A_w_q: jax.Array,
    A_w_uk: jax.Array,
    A_w_uv: jax.Array,
    A_w_o: jax.Array,
    B_x: jax.Array,
    B_w1: jax.Array,
    B_w2: jax.Array,
    c: jax.Array,
    w_mod: jax.Array,
    grad_out: jax.Array,
):
    del B_x
    sds = jax.ShapeDtypeStruct
    out_shape = (
        sds((S, M), bf16), sds((S, M), bf16), sds((S, M), bf16),
        sds((8, 16, 128, D), bf16), sds((8, 16, 128, D), bf16), sds((8, 16, 128, D), bf16),
        sds((H * D, M), bf16), sds((M, FF), bf16), sds((FF, M), bf16),
        sds((1, M), bf16), sds((M, 6 * M), bf16),
        sds((NSAVE, NTILE, 128, 128), bf16),
    )
    any_spec = pl.BlockSpec(memory_space=pl.ANY)
    outs = pl.pallas_call(
        _kernel,
        out_shape=out_shape,
        in_specs=[any_spec] * 11,
        out_specs=(any_spec,) * 12,
        scratch_shapes=[
            pltpu.VMEM((H, NT_, D, 128), bf16),
            pltpu.VMEM((2 * H, S, D), bf16),
            pltpu.VMEM((H, NT_, D, 128), bf16),
            pltpu.VMEM((WROWS, D), bf16),
            pltpu.VMEM((WROWS, D), bf16),
            pltpu.VMEM((WROWS, D), bf16),
            pltpu.VMEM((H, NTILE, 128), f32),
            pltpu.VMEM((H, 1, S), f32),
            pltpu.VMEM((1, 6 * M), f32),
            pltpu.VMEM((6, 8, M), f32),
            pltpu.VMEM((S, M), bf16),
            pltpu.VMEM((1, M), bf16),
            pltpu.VMEM((H * D, M), bf16),
            pltpu.SemaphoreType.DMA((NSEM,)),
        ],
        compiler_params=pltpu.CompilerParams(vmem_limit_bytes=128 * 1024 * 1024),
        name="adaln_block",
    )(A_x.reshape(S, M), A_c_kv.reshape(S, M), A_w_q, A_w_uk, A_w_uv,
      A_w_o.reshape(H * D, M),
      B_w1, B_w2, c, w_mod, grad_out.reshape(S, M))
    out, dx, dckv, dwq, dwuk, dwuv, dwo, dw1, dw2, dc, dwmod, _ = outs
    return (out.reshape(1, S, M), dx.reshape(1, S, M), dckv.reshape(1, S, M),
            dwq.reshape(M, H, D), dwuk.reshape(M, H, D), dwuv.reshape(M, H, D),
            dwo.reshape(H, D, M), dw1, dw2, dc, dwmod)
```
